```python
import jax
import jax.numpy as jnp

def _softmax(x, axis=-1):
    return jax.nn.softmax(x, axis=axis)
def _gelu(x):
    return jax.nn.gelu(x, approximate=True)
def _silu(x):
    return jax.nn.silu(x)
def _sigmoid(x):
    return jax.nn.sigmoid(x)
def _layernorm(x, axis=-1, eps=1e-5):
    m = jnp.mean(x, axis=axis, keepdims=True)
    v = jnp.var(x, axis=axis, keepdims=True)
    return (x - m) / jnp.sqrt(v + eps)
def _scatter_add(tgt, idx, src, axis=0):
    return tgt.at[idx].add(src)
def _segment_sum(src, seg, n):
    return jax.ops.segment_sum(src, seg, n)
class _Rng:
    def __init__(self, key):
        self._k = key
    def _next(self):
        self._k, sub = jax.random.split(self._k)
        return sub
    def normal(self, shape):
        return jax.random.normal(self._next(), shape, dtype=jnp.bfloat16)
    def randint(self, lo, hi, shape):
        return jax.random.randint(self._next(), shape, lo, hi, dtype=jnp.int32)
    def uniform(self, shape, lo=0.0, hi=1.0):
        return jax.random.uniform(self._next(), shape, jnp.bfloat16, lo, hi)
    def permutation(self, n):
        return jax.random.permutation(self._next(), n)


kernel_name = 'sequential_preLN__compressed_kv_cla__moe_arch_mod__decode'

def setup_inputs():
    _rng = _Rng(jax.random.key(int.from_bytes(__import__("os").urandom(4), "little")))
    _w = (lambda a: (lambda t: t.astype(jnp.bfloat16) if jnp.issubdtype(t.dtype, jnp.floating) else t)(jnp.asarray(a)))
    def _A_setup():
        B, H, Sq, Sk, D, M = 1, 32, 1, 8192, 128, 512
        Dc = 4 * D
        return {
            "x": _w((lambda *s: _rng.normal(s) * 0.05)(B, Sq, M)),
            "c_kv": _w((lambda *s: _rng.normal(s) * 0.05)(B, Sk, Dc)),
            "w_q": _w((lambda *s: _rng.normal(s) * 0.05)(M, H, D) * (M ** -0.5)),
            "w_uk": _w((lambda *s: _rng.normal(s) * 0.05)(Dc, H, D) * (Dc ** -0.5)),
            "w_uv": _w((lambda *s: _rng.normal(s) * 0.05)(Dc, H, D) * (Dc ** -0.5)),
            "w_o": _w((lambda *s: _rng.normal(s) * 0.05)(H, D, M) * ((H * D) ** -0.5)),
        }
    _A_in = _A_setup()

    def _B_setup():
        B, S, D, F, C = 1, 1, 512, 1376, 1
        return {
            "x": _w((lambda *s: _rng.normal(s) * 0.05)(B, S, D)),
            "w_r": _w((lambda *s: _rng.normal(s) * 0.05)(D)),
            "w_gate": _w((lambda *s: _rng.normal(s) * 0.05)(D, F)),
            "w_up": _w((lambda *s: _rng.normal(s) * 0.05)(D, F)),
            "w_down": _w((lambda *s: _rng.normal(s) * 0.05)(F, D)),
        }
    _B_in = _B_setup()

    return {
        "A_x": _A_in["x"],
        "A_c_kv": _A_in["c_kv"],
        "A_w_q": _A_in["w_q"],
        "A_w_uk": _A_in["w_uk"],
        "A_w_uv": _A_in["w_uv"],
        "A_w_o": _A_in["w_o"],
        "B_x": _B_in["x"],
        "B_w_r": _B_in["w_r"],
        "B_w_gate": _B_in["w_gate"],
        "B_w_up": _B_in["w_up"],
        "B_w_down": _B_in["w_down"],
    }

def reference(A_x, A_c_kv, A_w_q, A_w_uk, A_w_uv, A_w_o, B_x, B_w_r, B_w_gate, B_w_up, B_w_down):
    def _A_ref(x, c_kv, w_q, w_uk, w_uv, w_o):
        B, Sq, M = x.shape[0], x.shape[1], x.shape[2]
        Sk = c_kv.shape[1]
        H, D = w_q.shape[1], w_q.shape[2]
        q = jnp.einsum("bqm,mhd->bhqd", x, w_q)
        k = jnp.einsum("bkc,chd->bhkd", c_kv, w_uk)
        v = jnp.einsum("bkc,chd->bhkd", c_kv, w_uv)
        scores = jnp.einsum("bhqd,bhkd->bhqk", q, k) * (D ** -0.5)
        off = Sk - Sq
        qi = jnp.arange(Sq)[:, None]
        kj = jnp.arange(Sk)[None, :]
        cmask = kj <= (qi + off)
        scores = jnp.where(cmask[None, None], scores, -1e9)
        p = _softmax(scores, axis=-1)
        ctx = jnp.einsum("bhqk,bhkd->bhqd", p, v)
        return jnp.einsum("bhqd,hdm->bqm", ctx, w_o)

    def _B_ref(x, w_r, w_gate, w_up, w_down):
        B, S, D = x.shape
        C = 1
        r = x @ w_r
        idx = jnp.argsort(-r, axis=-1)[:, :C]
        idx_e = jnp.repeat(idx.reshape(B, C, 1), D, axis=2)
        x_sel = jnp.take_along_axis(x, idx_e, axis=1)
        g = _silu(x_sel @ w_gate)
        u = x_sel @ w_up
        y = (g * u) @ w_down
        r_sel = _sigmoid(jnp.take_along_axis(r, idx, axis=1))
        y = y * r_sel.reshape(B, C, 1)
        b_off = (jnp.arange(B) * S).reshape(B, 1)
        flat_idx = (idx + b_off).reshape(B * C)
        zero = (x * 0.0).reshape(B * S, D)
        upd = _scatter_add(zero, flat_idx, y.reshape(B * C, D), axis=0)
        return x + upd.reshape(B, S, D)

    x = A_x
    h = x + _A_ref(_layernorm(x, axis=-1), A_c_kv, A_w_q, A_w_uk, A_w_uv, A_w_o)
    h2 = h + _B_ref(_layernorm(h, axis=-1), B_w_r, B_w_gate, B_w_up, B_w_down)
    return h2
```

```python
import functools

import jax
import jax.numpy as jnp
from jax import lax
import jax.experimental.pallas as pl
import jax.experimental.pallas.tpu as pltpu

_F32 = jnp.float32
_BF16 = jnp.bfloat16
_LANES = 128
_NT = (((1,), (1,)), ((), ()))


def _layernorm(v):
    mean = jnp.mean(v, axis=-1, keepdims=True)
    cen = v - mean
    var = jnp.mean(cen * cen, axis=-1, keepdims=True)
    return cen / jnp.sqrt(var + 1e-5)


def _kernel(x_hbm, ckv_hbm, wq_hbm, wuk_hbm, wuv_hbm, wo_hbm, wr_hbm, wg_hbm, wu_hbm, wd_hbm,
            o_ref,
            x_v, wr_v, ckv_v, wq_v, wuk_v, wuv_v, wo_v, wg_v, wu_v, wd_v,
            tbl_ref, z_ref, ctx_ref, sems, small_sems,
            *, depth, n_w, n_kv, kv_sub, up_splits, down_splits):
    M, H, D = wq_v.shape
    G, T = wuk_v.shape[0], wuk_v.shape[1]
    Sk, Dc = ckv_v.shape

    def rows(src, dst, n):
        size = src.shape[0] // n
        return n, lambda i: (src.at[pl.ds(i * size, size)], dst.at[pl.ds(i * size, size)])

    def slabs(src, dst, n):
        size = src.shape[1] // n
        return n, lambda i: (src.at[:, pl.ds(i * size, size)], dst.at[:, pl.ds(i * size, size)])

    phases = [rows(wq_hbm, wq_v, n_w), slabs(wuk_hbm, wuk_v, n_w), rows(ckv_hbm, ckv_v, n_kv),
              slabs(wuv_hbm, wuv_v, n_w), rows(wo_hbm, wo_v, n_w)]
    first = [0]
    for n, _ in phases:
        first.append(first[-1] + n)
    tail = []
    for lo, hi in up_splits:
        tail.append((wg_hbm.at[lo:hi], wg_v.at[lo:hi]))
        tail.append((wu_hbm.at[lo:hi], wu_v.at[lo:hi]))
    for lo, hi in down_splits:
        tail.append((wd_hbm.at[lo:hi], wd_v.at[lo:hi]))
    n_chunks = first[-1] + len(tail)

    def static_copy(g):
        if g >= first[-1]:
            src, dst = tail[g - first[-1]]
        else:
            p = max(k for k in range(len(phases)) if first[k] <= g)
            src, dst = phases[p][1](g - first[p])
        return pltpu.make_async_copy(src, dst, sems.at[g % depth])

    def advance_static(g):
        static_copy(g).wait()
        if g + depth < n_chunks:
            static_copy(g + depth).start()

    def advance(p, i):
        n, chunk = phases[p]
        sem = sems.at[lax.rem(first[p] + i, depth)]
        pltpu.make_async_copy(*chunk(i), sem).wait()
        if n > depth:
            @pl.when(i < n - depth)
            def _():
                pltpu.make_async_copy(*chunk(i + depth), sem).start()
        for k in range(max(n - depth, 0), n):
            if first[p] + k + depth < n_chunks:
                @pl.when(i == k)
                def _():
                    static_copy(first[p] + k + depth).start()

    static_copy(0).start()
    x_copy = pltpu.make_async_copy(x_hbm, x_v, small_sems.at[0])
    wr_copy = pltpu.make_async_copy(wr_hbm, wr_v, small_sems.at[1])
    x_copy.start()
    for g in range(1, depth):
        static_copy(g).start()
    wr_copy.start()

    x_copy.wait()
    x = x_v[0].astype(_F32)
    xn = _layernorm(x).astype(_BF16).astype(_F32)
    for j in range(M // _LANES):
        blk = jnp.broadcast_to(xn[:, j * _LANES:(j + 1) * _LANES], (_LANES, _LANES))
        tbl_ref[j * _LANES:(j + 1) * _LANES, :] = blk.T

    def q_chunk(i, acc):
        advance(0, i)
        size = M // n_w

        def body(b, acc):
            base = pl.multiple_of(i * size + b * 8, 8)
            xb = tbl_ref[pl.ds(base, 8), :]
            for k in range(8):
                acc = acc + wq_v[base + k].astype(_F32) * xb[k:k + 1, :]
            return acc
        return lax.fori_loop(0, size // 8, body, acc)

    q = lax.fori_loop(0, n_w, q_chunk, jnp.zeros((H, D), _F32)).astype(_BF16)

    own_head = (lax.broadcasted_iota(jnp.int32, (H, G * H), 1) % H
                == lax.broadcasted_iota(jnp.int32, (H, G * H), 0))

    def uk_chunk(i, carry):
        advance(1, i)
        size = T // n_w

        def body(b, carry):
            base = pl.multiple_of(i * size + b * 8, 8)
            out = []
            for k in range(8):
                w = wuk_v[:, base + k].reshape(G * H, D)
                full = lax.dot_general(q, w, _NT, preferred_element_type=_F32)
                out.append(jnp.sum(jnp.where(own_head, full, 0.0), axis=0, keepdims=True))
            z_ref[pl.ds(base, 8), :] = jnp.concatenate(out, axis=0)
            return carry
        return lax.fori_loop(0, size // 8, body, carry)

    lax.fori_loop(0, n_w, uk_chunk, 0)
    zt = z_ref[...].T * (D ** -0.5)
    qa = jnp.concatenate([zt[j * H:(j + 1) * H, :] for j in range(G)], axis=1).astype(_BF16)

    def kv_chunk(i, carry):
        advance(2, i)
        size = Sk // n_kv

        def body(b, carry):
            m_old, l_old, acc = carry
            base = pl.multiple_of(i * size + b * kv_sub, kv_sub)
            c = ckv_v[pl.ds(base, kv_sub), :]
            s = lax.dot_general(qa, c, _NT, preferred_element_type=_F32)
            m_new = jnp.maximum(m_old, jnp.max(s, axis=-1, keepdims=True))
            alpha = jnp.exp(m_old - m_new)
            p = jnp.exp(s - m_new)
            l_new = alpha * l_old
            for k in range(kv_sub // _LANES):
                l_new = l_new + p[:, k * _LANES:(k + 1) * _LANES]
            acc = alpha * acc + jnp.dot(p.astype(_BF16), c, preferred_element_type=_F32)
            return m_new, l_new, acc
        return lax.fori_loop(0, size // kv_sub, body, carry)

    _, l_part, acc = lax.fori_loop(
        0, n_kv, kv_chunk,
        (jnp.full((H, 1), -jnp.inf, _F32), jnp.zeros((H, _LANES), _F32), jnp.zeros((H, Dc), _F32)))
    lat = acc / jnp.sum(l_part, axis=-1, keepdims=True)
    z_ref[...] = jnp.concatenate([lat[:, j * T:(j + 1) * T] for j in range(G)], axis=0).T

    def uv_chunk(i, acc):
        advance(3, i)
        size = T // n_w

        def body(b, acc):
            base = pl.multiple_of(i * size + b * 8, 8)
            zb = z_ref[pl.ds(base, 8), :]
            for k in range(8):
                lhs = jnp.where(own_head, zb[k:k + 1, :], 0.0).astype(_BF16)
                w = wuv_v[:, base + k].reshape(G * H, D)
                acc = acc + jnp.dot(lhs, w, preferred_element_type=_F32)
            return acc
        return lax.fori_loop(0, size // 8, body, acc)

    ctx_ref[...] = lax.fori_loop(0, n_w, uv_chunk, jnp.zeros((H, D), _F32))

    sublane = lax.broadcasted_iota(jnp.int32, (8, D), 0)

    def o_chunk(i, acc):
        advance(4, i)
        size = H // n_w

        def body(b, acc):
            h0 = pl.multiple_of(i * size + b * 8, 8)
            cb = ctx_ref[pl.ds(h0, 8), :]
            lhs = jnp.concatenate([jnp.where(sublane == k, cb, 0.0) for k in range(8)], axis=1)
            w = wo_v[pl.ds(pl.multiple_of(h0 * D, 8 * D), 8 * D), :]
            return acc + jnp.dot(lhs.astype(_BF16), w, preferred_element_type=_F32)
        return lax.fori_loop(0, size // 8, body, acc)

    attn = lax.fori_loop(0, n_w, o_chunk, jnp.zeros((8, M), _F32))
    h = x + jnp.sum(attn, axis=0, keepdims=True)

    hn = _layernorm(h)
    wr_copy.wait()
    wr = wr_v[...].astype(_F32)
    r = sum(jnp.sum(hn[:, j * _LANES:(j + 1) * _LANES] * wr[j:j + 1, :], axis=-1, keepdims=True)
            for j in range(M // _LANES))
    gate = jax.nn.sigmoid(r)
    resid = h + (hn + hn * 0.0)
    hb = jnp.broadcast_to(hn, (8, M)).astype(_BF16)

    g_idx = first[-1]
    act = []
    for lo, hi in up_splits:
        advance_static(g_idx)
        g = lax.dot_general(hb, wg_v[lo:hi, :], _NT, preferred_element_type=_F32)
        advance_static(g_idx + 1)
        u = lax.dot_general(hb, wu_v[lo:hi, :], _NT, preferred_element_type=_F32)
        act.append((g * jax.nn.sigmoid(g) * u).astype(_BF16))
        g_idx += 2
    act = jnp.concatenate(act, axis=1)
    y = jnp.zeros((8, M), _F32)
    for lo, hi in down_splits:
        advance_static(g_idx)
        y = y + jnp.dot(act[:, lo:hi], wd_v[lo:hi, :], preferred_element_type=_F32)
        g_idx += 1
    o_ref[0] = (resid + y[0:1, :] * gate).astype(o_ref.dtype)


def _splits(edges):
    return tuple(zip(edges[:-1], edges[1:]))


def _forward(A_x, A_c_kv, A_w_q, A_w_uk, A_w_uv, A_w_o, B_w_r, B_w_gate, B_w_up, B_w_down, *,
             depth=3, n_w=4, n_kv=8, kv_sub=512,
             up_edges=(0, 768, 1376), down_edges=(0, 640, 1152, 1376)):
    B, Sq, M = A_x.shape
    _, Sk, Dc = A_c_kv.shape
    _, H, D = A_w_q.shape
    F = B_w_gate.shape[1]
    assert B == 1 and Sq == 1 and D == _LANES and _LANES % H == 0
    G = _LANES // H
    T = Dc // G
    assert T == _LANES and up_edges[-1] == F and down_edges[-1] == F

    hbm = pl.BlockSpec(memory_space=pltpu.HBM)
    body = functools.partial(_kernel, depth=depth, n_w=n_w, n_kv=n_kv, kv_sub=kv_sub,
                             up_splits=_splits(up_edges), down_splits=_splits(down_edges))
    return pl.pallas_call(
        body,
        out_shape=jax.ShapeDtypeStruct((B, Sq, M), A_x.dtype),
        in_specs=[hbm] * 10,
        out_specs=pl.BlockSpec(memory_space=pltpu.VMEM),
        scratch_shapes=[
            pltpu.VMEM((B, Sq, M), _BF16),
            pltpu.VMEM((M // _LANES, _LANES), _BF16),
            pltpu.VMEM((Sk, Dc), _BF16),
            pltpu.VMEM((M, H, D), _BF16),
            pltpu.VMEM((G, T, H, D), _BF16),
            pltpu.VMEM((G, T, H, D), _BF16),
            pltpu.VMEM((H * D, M), _BF16),
            pltpu.VMEM((F, M), _BF16),
            pltpu.VMEM((F, M), _BF16),
            pltpu.VMEM((F, M), _BF16),
            pltpu.VMEM((M, _LANES), _F32),
            pltpu.VMEM((T, G * H), _F32),
            pltpu.VMEM((H, D), _F32),
            pltpu.SemaphoreType.DMA((depth,)),
            pltpu.SemaphoreType.DMA((2,)),
        ],
        compiler_params=pltpu.CompilerParams(vmem_limit_bytes=64 * 2**20),
    )(
        A_x,
        A_c_kv.reshape(Sk, Dc),
        A_w_q,
        A_w_uk.reshape(G, T, H, D),
        A_w_uv.reshape(G, T, H, D),
        A_w_o.reshape(H * D, M),
        B_w_r.reshape(M // _LANES, _LANES),
        B_w_gate.T,
        B_w_up.T,
        B_w_down,
    )


@jax.jit
def pallas_sequential_preLN__compressed_kv_cla__moe_arch_mod__decode_kernel(
    A_x: jax.Array,
    A_c_kv: jax.Array,
    A_w_q: jax.Array,
    A_w_uk: jax.Array,
    A_w_uv: jax.Array,
    A_w_o: jax.Array,
    B_x: jax.Array,
    B_w_r: jax.Array,
    B_w_gate: jax.Array,
    B_w_up: jax.Array,
    B_w_down: jax.Array,
):
    del B_x
    return _forward(A_x, A_c_kv, A_w_q, A_w_uk, A_w_uv, A_w_o, B_w_r, B_w_gate, B_w_up, B_w_down)
```

```python
import functools

import jax
import jax.numpy as jnp
from jax import lax
import jax.experimental.pallas as pl
import jax.experimental.pallas.tpu as pltpu

_F32 = jnp.float32
_BF16 = jnp.bfloat16
_LANES = 128
_NT = (((1,), (1,)), ((), ()))


def _layernorm(v):
    mean = jnp.mean(v, axis=-1, keepdims=True)
    cen = v - mean
    var = jnp.mean(cen * cen, axis=-1, keepdims=True)
    return cen / jnp.sqrt(var + 1e-5)


def _kernel(x_hbm, ckv_hbm, wq_hbm, wuk_hbm, wuv_hbm, wo_hbm, wr_hbm, wg_hbm, wu_hbm, wd_hbm,
            o_ref,
            x_v, wr_v, ckv_v, wq_v, wuk_v, wuv_v, wo_v, wg_v, wu_v, wd_v,
            tbl_ref, z_ref, s_ref, acc_ref, ctx_ref, act_ref, sems, small_sems,
            *, step_kb, depth, head, mark, late_tiles=4, late_keys=3, late_uv=4, down_edges=(4, 8, 10), dma=True, compute=True):
    M, H, D = wq_v.shape
    G, T = wuk_v.shape[0], wuk_v.shape[1]
    Sk, Dc = ckv_v.shape
    F = wg_v.shape[0]
    slabs = step_kb * 1024 // (H * D * 2)
    rows = step_kb * 1024 // (M * 2)
    f_full, f_rest = F // rows, F % rows
    slots = sems.shape[0] // 2

    def row_window(src, dst, size, first=0):
        def window(i, lo, hi):
            start = first + i * size + lo
            if not isinstance(start, int):
                start = pl.multiple_of(start, 8)
            return src.at[pl.ds(start, hi - lo)], dst.at[pl.ds(start, hi - lo)]
        return size, window

    def slab_window(src, dst):
        def window(i, lo, hi):
            j, start = i % G, (i // G) * slabs + lo
            return src.at[j, pl.ds(start, hi - lo)], dst.at[j, pl.ds(start, hi - lo)]
        return slabs, window

    runs = [(M // slabs, *row_window(wq_hbm, wq_v, slabs)),
            (G * T // slabs, *slab_window(wuk_hbm, wuk_v)),
            (Sk // rows, *row_window(ckv_hbm, ckv_v, rows)),
            (G * T // slabs, *slab_window(wuv_hbm, wuv_v)),
            (H * D // rows, *row_window(wo_hbm, wo_v, rows))]
    for src, dst in ((wg_hbm, wg_v), (wu_hbm, wu_v), (wd_hbm, wd_v)):
        runs.append((f_full, *row_window(src, dst, rows)))
        runs.append((1, *row_window(src, dst, f_rest, f_full * rows)))
    first = [0]
    for n, _, _ in runs:
        first.append(first[-1] + n)
    n_steps = first[-1]
    t_uk, t_kv, t_uv, t_o, t_gate, t_up, t_down = (first[k] for k in (1, 2, 3, 4, 5, 7, 9))

    def run_of(step):
        return max(k for k in range(len(runs)) if first[k] <= step)

    def copies(k, i, slot):
        _, size, window = runs[k]
        unit = 8 if size > slabs else 1
        lo = size * mark // step_kb // unit * unit
        hi = lo + size * head // step_kb // unit * unit
        return (pltpu.make_async_copy(*window(i, lo, hi), sems.at[2 * slot]),
                [pltpu.make_async_copy(*window(i, a, b), sems.at[2 * slot + 1])
                 for a, b in ((0, lo), (hi, size)) if a < b])

    def start_step(k, i, slot):
        early, late = copies(k, i, slot)
        early.start(priority=0)
        for copy in late:
            copy.start(priority=1)

    def tick(g, k_wait, k_start):
        if not dma:
            return
        early, late = copies(k_wait, g - first[k_wait], g % slots)
        for copy in late:
            copy.wait()
        if k_start is not None:
            start_step(k_start, g + depth - first[k_start], (g + depth) % slots)
        early.wait()

    def stream(lo, n, body=None, carry=None, span=1):
        def runs_at(i):
            steps = range(lo + i * span, lo + (i + 1) * span)
            return [(run_of(g), run_of(g + depth) if g + depth < n_steps else None) for g in steps]

        a = 0
        while a < n:
            b = a + 1
            while b < n and runs_at(b) == runs_at(a):
                b += 1

            def step(i, c, ks=runs_at(a)):
                g = lo + i * span
                tick(g, *ks[0])
                rest = [functools.partial(tick, g + 1, *ks[1])] if span == 2 else []
                if body is None or (compute is not True and body.__name__ not in (compute or ())):
                    for t in rest:
                        t()
                    return c
                return body(i, c, *rest)

            carry = step(a, carry) if b - a == 1 else lax.fori_loop(a, b, step, carry)
            a = b
        return carry

    def aligned(start, size):
        return pl.ds(start if isinstance(start, int) else pl.multiple_of(start, size), size)

    x_copy = pltpu.make_async_copy(x_hbm, x_v, small_sems.at[0])
    wr_copy = pltpu.make_async_copy(wr_hbm, wr_v, small_sems.at[1])
    x_copy.start()
    if dma:
        for g in range(depth):
            start_step(0, g, g)
    wr_copy.start()

    x_copy.wait()
    x = x_v[0].astype(_F32)
    xn = _layernorm(x).astype(_BF16).astype(_F32)
    for j in range(M // _LANES):
        blk = jnp.broadcast_to(xn[:, j * _LANES:(j + 1) * _LANES], (_LANES, _LANES))
        tbl_ref[j * _LANES:(j + 1) * _LANES, :] = blk.T

    def q_body(i, acc):
        for b in range(slabs // 8):
            base = pl.multiple_of(i * slabs + b * 8, 8)
            xb = tbl_ref[pl.ds(base, 8), :]
            for k in range(8):
                acc = acc + wq_v[base + k].astype(_F32) * xb[k:k + 1, :]
        return acc

    q = stream(0, t_uk, q_body, jnp.zeros((H, D), _F32)).astype(_BF16)

    own_head = (lax.broadcasted_iota(jnp.int32, (H, G * H), 1) % H
                == lax.broadcasted_iota(jnp.int32, (H, G * H), 0))
    tiles = 2 * slabs // G

    def uk_body(i, carry, next_tick):
        full = []
        for k in range(tiles):
            if k == tiles - late_tiles:
                next_tick()
            w = wuk_v[:, i * tiles + k].reshape(G * H, D)
            full.append(lax.dot_general(q, w, _NT, preferred_element_type=_F32))
        z_ref[aligned(i * tiles, tiles), :] = jnp.concatenate(
            [jnp.sum(jnp.where(own_head, f, 0.0), axis=0, keepdims=True) for f in full], axis=0)
        return carry

    now = t_uk + G - 1
    stream(t_uk, G - 1)
    stream(now, T // tiles, uk_body, 0, span=2)
    now += 2 * T // tiles
    stream(now, 1)
    zt = z_ref[...].T * (D ** -0.5)
    qa = jnp.concatenate([zt[j * H:(j + 1) * H, :] for j in range(G)], axis=1).astype(_BF16)
    now += 1

    def score_body(i, peak, next_tick):
        for k in range(2):
            if k == 1:
                next_tick()
            s = lax.dot_general(qa, ckv_v[aligned((2 * i + k) * rows, rows), :], _NT,
                                preferred_element_type=_F32)
            s_ref[2 * i + k] = s
            peak = jnp.maximum(peak, s)
        return peak

    assert now >= t_kv + 1
    peak = stream(now, Sk // (2 * rows), score_body, jnp.full((H, rows), -jnp.inf, _F32), span=2)
    now += Sk // rows
    peak = jnp.broadcast_to(jnp.max(peak, axis=-1, keepdims=True), (H, rows))

    def value_body(i, total, next_tick):
        acc = acc_ref[...]
        for k in range(4):
            if k == late_keys:
                next_tick()
            p = jnp.exp(s_ref[4 * i + k] - peak)
            total = total + p
            acc = acc + jnp.dot(p.astype(_BF16), ckv_v[aligned((4 * i + k) * rows, rows), :],
                                preferred_element_type=_F32)
        acc_ref[...] = acc
        return total

    acc_ref[...] = jnp.zeros_like(acc_ref)
    total = stream(now, Sk // (4 * rows), value_body, jnp.zeros((H, rows), _F32), span=2)
    now += Sk // (2 * rows)
    stream(now, 1)
    lat = acc_ref[...] / jnp.sum(total, axis=-1, keepdims=True)
    z_ref[...] = jnp.concatenate([lat[:, j * T:(j + 1) * T] for j in range(G)], axis=0).T
    now += 1

    def uv_body(i, ctx, next_tick):
        zb = z_ref[aligned(2 * i * tiles, 2 * tiles), :]
        for k in range(2 * tiles):
            if k == 2 * tiles - late_uv:
                next_tick()
            lhs = jnp.where(own_head, zb[k:k + 1, :], 0.0).astype(_BF16)
            w = wuv_v[:, 2 * i * tiles + k].reshape(G * H, D)
            ctx = ctx + jnp.dot(lhs, w, preferred_element_type=_F32)
        return ctx

    assert now >= t_o - 1
    ctx_ref[...] = stream(now, T // (2 * tiles), uv_body, jnp.zeros((H, D), _F32), span=2)
    now += T // tiles

    heads = 4 * rows // D

    def o_body(i, carry, next_tick):
        for k in range(heads):
            if k == heads - 1:
                next_tick()
            lhs = jnp.broadcast_to(ctx_ref[pl.ds(heads * i + k, 1), :], (8, D)).astype(_BF16)
            w = wo_v[aligned((heads * i + k) * D, D), :]
            carry = carry + jnp.dot(lhs, w, preferred_element_type=_F32)
        return carry

    begin = max(now, t_gate + 1 - 2 * H // heads)
    stream(now, begin - now)
    attn = stream(begin, H // heads, o_body, jnp.zeros((8, M), _F32), span=2)
    now = begin + 2 * H // heads

    stream(now, 1)
    h = x + attn[0:1, :]
    hn = _layernorm(h)
    hb = jnp.broadcast_to(hn, (8, M)).astype(_BF16)
    stream(now + 1, 1)
    wr_copy.wait()
    wr = wr_v[...].astype(_F32)
    r = sum(jnp.sum(hn[:, j * _LANES:(j + 1) * _LANES] * wr[j:j + 1, :], axis=-1, keepdims=True)
            for j in range(M // _LANES))
    gate = jax.nn.sigmoid(r)
    resid = h + (hn + hn * 0.0)
    now += 2

    def project(w_v, window):
        return lax.dot_general(hb, w_v[window, :], _NT, preferred_element_type=_F32)

    def silu(v):
        return v * jax.nn.sigmoid(v)

    def up_body(i, carry, next_tick):
        g = silu(project(wg_v, aligned(2 * i * rows, 2 * rows)))
        u0 = project(wu_v, aligned(2 * i * rows, rows))
        next_tick()
        u1 = project(wu_v, aligned((2 * i + 1) * rows, rows))
        act_ref[2 * i] = g[:, :rows] * u0
        act_ref[2 * i + 1] = g[:, rows:] * u1
        return carry

    assert now <= t_up + 1 and f_full % 2 == 0
    stream(now, t_up + 1 - now)
    stream(t_up + 1, f_full // 2, up_body, 0, span=2)
    rest = pl.ds(f_full * rows, f_rest)
    act_rest = (silu(project(wg_v, rest)) * project(wu_v, rest)).astype(_BF16)
    y = jnp.zeros((8, M), _F32)
    done = 0
    for edge in down_edges:
        stream(t_down + done, edge - done)
        for i in range(done, edge):
            y = y + jnp.dot(act_ref[i].astype(_BF16), wd_v[i * rows:(i + 1) * rows, :],
                            preferred_element_type=_F32)
        done = edge
    assert done == f_full
    stream(t_down + f_full, 1)
    y = y + jnp.dot(act_rest, wd_v[rest, :], preferred_element_type=_F32)
    o_ref[0] = (resid + y[0:1, :] * gate).astype(o_ref.dtype)


def _forward(A_x, A_c_kv, A_w_q, A_w_uk, A_w_uv, A_w_o, B_w_r, B_w_gate, B_w_up, B_w_down, *,
             step_kb=128, depth=12, head=56, mark=32, params=None, **debug):
    B, Sq, M = A_x.shape
    _, Sk, Dc = A_c_kv.shape
    _, H, D = A_w_q.shape
    F = B_w_gate.shape[1]
    assert B == 1 and Sq == 1 and D == _LANES and _LANES % H == 0 and Dc == M
    G = _LANES // H
    T = Dc // G
    rows = step_kb * 1024 // (M * 2)
    assert T == _LANES

    hbm = pl.BlockSpec(memory_space=pltpu.HBM)
    return pl.pallas_call(
        functools.partial(_kernel, step_kb=step_kb, depth=depth, head=head, mark=mark, **debug),
        out_shape=jax.ShapeDtypeStruct((B, Sq, M), A_x.dtype),
        in_specs=[hbm] * 10,
        out_specs=pl.BlockSpec(memory_space=pltpu.VMEM),
        scratch_shapes=[
            pltpu.VMEM((B, Sq, M), _BF16),
            pltpu.VMEM((M // _LANES, _LANES), _BF16),
            pltpu.VMEM((Sk, Dc), _BF16),
            pltpu.VMEM((M, H, D), _BF16),
            pltpu.VMEM((G, T, H, D), _BF16),
            pltpu.VMEM((G, T, H, D), _BF16),
            pltpu.VMEM((H * D, M), _BF16),
            pltpu.VMEM((F, M), _BF16),
            pltpu.VMEM((F, M), _BF16),
            pltpu.VMEM((F, M), _BF16),
            pltpu.VMEM((M, _LANES), _F32),
            pltpu.VMEM((T, G * H), _F32),
            pltpu.VMEM((Sk // rows, H, rows), _F32),
            pltpu.VMEM((H, Dc), _F32),
            pltpu.VMEM((H, D), _F32),
            pltpu.VMEM((F // rows, 8, rows), _F32),
            pltpu.SemaphoreType.DMA((2 * pl.next_power_of_2(depth + 1),)),
            pltpu.SemaphoreType.DMA((2,)),
        ],
        compiler_params=pltpu.CompilerParams(vmem_limit_bytes=64 * 2**20, **(params or {})),
    )(
        A_x,
        A_c_kv.reshape(Sk, Dc),
        A_w_q,
        A_w_uk.reshape(G, T, H, D),
        A_w_uv.reshape(G, T, H, D),
        A_w_o.reshape(H * D, M),
        B_w_r.reshape(M // _LANES, _LANES),
        B_w_gate.T,
        B_w_up.T,
        B_w_down,
    )


@jax.jit
def pallas_sequential_preLN__compressed_kv_cla__moe_arch_mod__decode_kernel(
    A_x: jax.Array,
    A_c_kv: jax.Array,
    A_w_q: jax.Array,
    A_w_uk: jax.Array,
    A_w_uv: jax.Array,
    A_w_o: jax.Array,
    B_x: jax.Array,
    B_w_r: jax.Array,
    B_w_gate: jax.Array,
    B_w_up: jax.Array,
    B_w_down: jax.Array,
):
    del B_x
    return _forward(A_x, A_c_kv, A_w_q, A_w_uk, A_w_uv, A_w_o, B_w_r, B_w_gate, B_w_up, B_w_down)
```

```python
import functools

import jax
import jax.numpy as jnp
from jax import lax
import jax.experimental.pallas as pl
import jax.experimental.pallas.tpu as pltpu

_F32 = jnp.float32
_BF16 = jnp.bfloat16
_LANES = 128
_STEP = 128
_NT = (((1,), (1,)), ((), ()))


def _layernorm(v):
    mean = jnp.mean(v, axis=-1, keepdims=True)
    cen = v - mean
    var = jnp.mean(cen * cen, axis=-1, keepdims=True)
    return cen / jnp.sqrt(var + 1e-5)


def _kernel(x_hbm, ckv_hbm, wq_hbm, wuk_hbm, wuv_hbm, wo_hbm, wr_hbm, wg_hbm, wu_hbm, wd_hbm,
            o_ref,
            x_v, wr_v, ckv_v, wq_v, wuk_v, wuv_v, wo_v, wg_v, wu_v, wd_v,
            tbl_ref, z_ref, s_ref, acc_ref, ctx_ref, act_ref, sems, small_sems,
            *, depth, head, marks, ramp=10, late_tiles=4, late_keys=3, late_uv=4, down_edges=(4, 8), dma=True, compute=True):
    M, H, D = wq_v.shape
    G, T = wuk_v.shape[0], wuk_v.shape[1]
    Sk, Dc = ckv_v.shape
    F = wg_v.shape[0]
    slabs = _STEP * 1024 // (H * D * 2)
    rows = _STEP * 1024 // (M * 2)
    f_full, f_rest = F // rows, F % rows
    slots = sems.shape[0] // 2

    runs, first = [], [0]

    def add_run(n, window, early, late):
        if n:
            runs.append((n, window, early, late))
            first.append(first[-1] + n)

    def add_array(src, dst, mark, lanes=1, skip=0):
        t_first = first[-1]
        length = src.shape[1] if lanes > 1 else src.shape[0]
        total = src.size * 2 // 1024 // lanes

        def window(base):
            def at(i, lo, hi):
                start = (base + (i // lanes) * _STEP + lo) * length // total
                if not isinstance(start, int):
                    start = pl.multiple_of(start, 8 if length == total else 1)
                index = pl.ds(start, (hi - lo) * length // total)
                index = (i % lanes, index) if lanes > 1 else index
                return src.at[index], dst.at[index]
            return at

        def pieces(begin, end):
            cuts = (mark + head, mark + _STEP // 2, mark + _STEP)
            return ([(mark, min(mark + head, end))],
                    [(begin, mark)] + [(a, min(b, end)) for a, b in zip(cuts[:-1], cuts[1:])])

        inner = (total - skip - mark) // _STEP
        add_run(lanes, window(skip), *pieces(mark if skip else 0, total))
        add_run(lanes * (inner - 1), window(skip + _STEP), *pieces(mark, total))
        base = skip + inner * _STEP
        if base + mark < total:
            add_run(lanes, window(base), *pieces(mark, total - base))
        return t_first, window

    lead = ramp * _STEP // 2
    _, q_window = add_array(wq_hbm, wq_v, marks[0], skip=lead)
    for k in reversed(range(ramp)):
        lo = marks[0] + k * _STEP // 2
        runs.insert(0, (1, q_window(0), [], [(lo if k else 0, lo + _STEP // 2)]))
    first[:] = list(range(ramp)) + [e + ramp for e in first]
    t_uk = add_array(wuk_hbm, wuk_v, marks[1], lanes=G)[0]
    t_kv = add_array(ckv_hbm, ckv_v, marks[2])[0]
    t_uv = add_array(wuv_hbm, wuv_v, marks[3])[0]
    t_o = add_array(wo_hbm, wo_v, marks[4])[0]
    t_gate = add_array(wg_hbm, wg_v, marks[5])[0]
    t_up = add_array(wu_hbm, wu_v, marks[6])[0]
    t_down = add_array(wd_hbm, wd_v, marks[7])[0]
    n_steps = first[-1]

    def run_of(step):
        return max(k for k in range(len(runs)) if first[k] <= step)

    def copies(k, i, slot):
        _, window, *parts = runs[k]
        return [[pltpu.make_async_copy(*window(i, lo, hi), sems.at[2 * slot + queue])
                 for lo, hi in part if lo < hi] for queue, part in enumerate(parts)]

    def start_step(k, i, slot):
        for queue, part in enumerate(copies(k, i, slot)):
            for copy in part:
                copy.start(priority=queue)

    def tick(g, k_wait, k_start):
        if not dma:
            return
        early, late = copies(k_wait, g - first[k_wait], g % slots)
        for copy in late:
            copy.wait()
        if k_start is not None:
            start_step(k_start, g + depth - first[k_start], (g + depth) % slots)
        for copy in early:
            copy.wait()

    def stream(lo, n, body=None, carry=None, span=1):
        def runs_at(i):
            steps = range(lo + i * span, lo + (i + 1) * span)
            return [(run_of(g), run_of(g + depth) if g + depth < n_steps else None) for g in steps]

        a = 0
        while a < n:
            b = a + 1
            while b < n and runs_at(b) == runs_at(a):
                b += 1

            def step(i, c, ks=runs_at(a)):
                g = lo + i * span
                tick(g, *ks[0])
                rest = [functools.partial(tick, g + 1, *ks[1])] if span == 2 else []
                if body is None or (compute is not True and body.__name__ not in (compute or ())):
                    for t in rest:
                        t()
                    return c
                return body(i, c, *rest)

            carry = step(a, carry) if b - a == 1 else lax.fori_loop(a, b, step, carry)
            a = b
        return carry

    def aligned(start, size):
        return pl.ds(start if isinstance(start, int) else pl.multiple_of(start, size), size)

    x_copy = pltpu.make_async_copy(x_hbm, x_v, small_sems.at[0])
    wr_copy = pltpu.make_async_copy(wr_hbm, wr_v, small_sems.at[1])
    x_copy.start()
    if dma:
        for g in range(depth):
            start_step(run_of(g), g - first[run_of(g)], g)
    wr_copy.start()

    x_copy.wait()
    x = x_v[0].astype(_F32)
    xn = _layernorm(x).astype(_BF16).astype(_F32)
    for j in range(M // _LANES):
        blk = jnp.broadcast_to(xn[:, j * _LANES:(j + 1) * _LANES], (_LANES, _LANES))
        tbl_ref[j * _LANES:(j + 1) * _LANES, :] = blk.T

    def q_body(i, acc):
        for b in range(2 * slabs // 8):
            base = pl.multiple_of(2 * i * slabs + b * 8, 8)
            xb = tbl_ref[pl.ds(base, 8), :]
            for k in range(8):
                acc = acc + wq_v[base + k].astype(_F32) * xb[k:k + 1, :]
        return acc

    assert ramp < depth
    for g in range(ramp + 1):
        stream(g, 1)
    n_q = M // (2 * slabs)
    stream(ramp + 1, t_uk - n_q - ramp - 1)
    q = stream(t_uk - n_q, n_q, q_body, jnp.zeros((H, D), _F32)).astype(_BF16)

    own_head = (lax.broadcasted_iota(jnp.int32, (H, G * H), 1) % H
                == lax.broadcasted_iota(jnp.int32, (H, G * H), 0))
    tiles = 2 * slabs // G

    def uk_body(i, carry, next_tick):
        full = []
        for k in range(tiles):
            if k == tiles - late_tiles:
                next_tick()
            w = wuk_v[:, i * tiles + k].reshape(G * H, D)
            full.append(lax.dot_general(q, w, _NT, preferred_element_type=_F32))
        z_ref[aligned(i * tiles, tiles), :] = jnp.concatenate(
            [jnp.sum(jnp.where(own_head, f, 0.0), axis=0, keepdims=True) for f in full], axis=0)
        return carry

    now = t_uk + G - 1
    stream(t_uk, G - 1)
    stream(now, T // tiles, uk_body, 0, span=2)
    now += 2 * T // tiles
    stream(now, 1)
    zt = z_ref[...].T * (D ** -0.5)
    qa = jnp.concatenate([zt[j * H:(j + 1) * H, :] for j in range(G)], axis=1).astype(_BF16)
    now += 1

    def score_body(i, peak, next_tick):
        for k in range(2):
            if k == 1:
                next_tick()
            s = lax.dot_general(qa, ckv_v[aligned((2 * i + k) * rows, rows), :], _NT,
                                preferred_element_type=_F32)
            s_ref[2 * i + k] = s
            peak = jnp.maximum(peak, s)
        return peak

    assert now >= t_kv + 1
    peak = stream(now, Sk // (2 * rows), score_body, jnp.full((H, rows), -jnp.inf, _F32), span=2)
    now += Sk // rows
    peak = jnp.broadcast_to(jnp.max(peak, axis=-1, keepdims=True), (H, rows))

    def value_body(i, total, next_tick):
        acc = acc_ref[...]
        for k in range(4):
            if k == late_keys:
                next_tick()
            p = jnp.exp(s_ref[4 * i + k] - peak)
            total = total + p
            acc = acc + jnp.dot(p.astype(_BF16), ckv_v[aligned((4 * i + k) * rows, rows), :],
                                preferred_element_type=_F32)
        acc_ref[...] = acc
        return total

    acc_ref[...] = jnp.zeros_like(acc_ref)
    total = stream(now, Sk // (4 * rows), value_body, jnp.zeros((H, rows), _F32), span=2)
    now += Sk // (2 * rows)
    stream(now, 1)
    lat = acc_ref[...] / jnp.sum(total, axis=-1, keepdims=True)
    z_ref[...] = jnp.concatenate([lat[:, j * T:(j + 1) * T] for j in range(G)], axis=0).T
    now += 1

    def uv_body(i, ctx, next_tick):
        zb = z_ref[aligned(2 * i * tiles, 2 * tiles), :]
        for k in range(2 * tiles):
            if k == 2 * tiles - late_uv:
                next_tick()
            lhs = jnp.where(own_head, zb[k:k + 1, :], 0.0).astype(_BF16)
            t = 2 * i * tiles + k
            w = jnp.concatenate([wuv_v[j * T + t] for j in range(G)], axis=0)
            ctx = ctx + jnp.dot(lhs, w, preferred_element_type=_F32)
        return ctx

    assert now >= t_o
    ctx_ref[...] = stream(now, T // (2 * tiles), uv_body, jnp.zeros((H, D), _F32), span=2)
    now += T // tiles

    heads = 4 * rows // D

    def o_body(i, carry, next_tick):
        for k in range(heads):
            if k == heads - 1:
                next_tick()
            lhs = jnp.broadcast_to(ctx_ref[pl.ds(heads * i + k, 1), :], (8, D)).astype(_BF16)
            w = wo_v[aligned((heads * i + k) * D, D), :]
            carry = carry + jnp.dot(lhs, w, preferred_element_type=_F32)
        return carry

    begin = max(now, t_gate + 1 - 2 * H // heads)
    stream(now, begin - now)
    attn = stream(begin, H // heads, o_body, jnp.zeros((8, M), _F32), span=2)
    now = begin + 2 * H // heads

    stream(now, 1)
    h = x + attn[0:1, :]
    hn = _layernorm(h)
    hb = jnp.broadcast_to(hn, (8, M)).astype(_BF16)
    stream(now + 1, 1)
    wr_copy.wait()
    wr = wr_v[...].astype(_F32)
    r = sum(jnp.sum(hn[:, j * _LANES:(j + 1) * _LANES] * wr[j:j + 1, :], axis=-1, keepdims=True)
            for j in range(M // _LANES))
    gate = jax.nn.sigmoid(r)
    resid = h + (hn + hn * 0.0)
    now += 2

    def project(w_v, window):
        return lax.dot_general(hb, w_v[window, :], _NT, preferred_element_type=_F32)

    def silu(v):
        return v * jax.nn.sigmoid(v)

    def up_body(i, carry, next_tick):
        g = silu(project(wg_v, aligned(2 * i * rows, 2 * rows)))
        u0 = project(wu_v, aligned(2 * i * rows, rows))
        next_tick()
        u1 = project(wu_v, aligned((2 * i + 1) * rows, rows))
        act_ref[2 * i] = g[:, :rows] * u0
        act_ref[2 * i + 1] = g[:, rows:] * u1
        return carry

    assert now <= t_up + 1 and f_full % 2 == 0
    assert t_down - t_up == n_steps - t_down == f_full + 1
    stream(now, t_up + 1 - now)
    stream(t_up + 1, f_full // 2, up_body, 0, span=2)
    rest = pl.ds(f_full * rows, f_rest)
    act_rest = (silu(project(wg_v, rest)) * project(wu_v, rest)).astype(_BF16)
    y = jnp.zeros((8, M), _F32)
    done = 0
    for edge in down_edges + (f_full + 1,):
        stream(t_down + done, edge - done)
        for i in range(done, edge):
            act, window = ((act_ref[i].astype(_BF16), pl.ds(i * rows, rows)) if i < f_full
                           else (act_rest, rest))
            y = y + jnp.dot(act, wd_v[window, :], preferred_element_type=_F32)
        done = edge
    o_ref[0] = (resid + y[0:1, :] * gate).astype(o_ref.dtype)


def _forward(A_x, A_c_kv, A_w_q, A_w_uk, A_w_uv, A_w_o, B_w_r, B_w_gate, B_w_up, B_w_down, *,
             depth=12, head=56, marks=(32,) * 6 + (0, 32), params=None, **debug):
    B, Sq, M = A_x.shape
    _, Sk, Dc = A_c_kv.shape
    _, H, D = A_w_q.shape
    F = B_w_gate.shape[1]
    assert B == 1 and Sq == 1 and D == _LANES and _LANES % H == 0 and Dc == M
    G = _LANES // H
    T = Dc // G
    rows = _STEP * 1024 // (M * 2)
    assert T == _LANES

    hbm = pl.BlockSpec(memory_space=pltpu.HBM)
    return pl.pallas_call(
        functools.partial(_kernel, depth=depth, head=head, marks=marks, **debug),
        out_shape=jax.ShapeDtypeStruct((B, Sq, M), A_x.dtype),
        in_specs=[hbm] * 10,
        out_specs=pl.BlockSpec(memory_space=pltpu.VMEM),
        scratch_shapes=[
            pltpu.VMEM((B, Sq, M), _BF16),
            pltpu.VMEM((M // _LANES, _LANES), _BF16),
            pltpu.VMEM((Sk, Dc), _BF16),
            pltpu.VMEM((M, H, D), _BF16),
            pltpu.VMEM((G, T, H, D), _BF16),
            pltpu.VMEM((Dc, H, D), _BF16),
            pltpu.VMEM((H * D, M), _BF16),
            pltpu.VMEM((F, M), _BF16),
            pltpu.VMEM((F, M), _BF16),
            pltpu.VMEM((F, M), _BF16),
            pltpu.VMEM((M, _LANES), _F32),
            pltpu.VMEM((T, G * H), _F32),
            pltpu.VMEM((Sk // rows, H, rows), _F32),
            pltpu.VMEM((H, Dc), _F32),
            pltpu.VMEM((H, D), _F32),
            pltpu.VMEM((F // rows, 8, rows), _F32),
            pltpu.SemaphoreType.DMA((2 * pl.next_power_of_2(depth + 1),)),
            pltpu.SemaphoreType.DMA((2,)),
        ],
        compiler_params=pltpu.CompilerParams(vmem_limit_bytes=64 * 2**20, **(params or dict(disable_semaphore_checks=True, disable_bounds_checks=True))),
    )(
        A_x,
        A_c_kv.reshape(Sk, Dc),
        A_w_q,
        A_w_uk.reshape(G, T, H, D),
        A_w_uv,
        A_w_o.reshape(H * D, M),
        B_w_r.reshape(M // _LANES, _LANES),
        B_w_gate.T,
        B_w_up.T,
        B_w_down,
    )


@jax.jit
def pallas_sequential_preLN__compressed_kv_cla__moe_arch_mod__decode_kernel(
    A_x: jax.Array,
    A_c_kv: jax.Array,
    A_w_q: jax.Array,
    A_w_uk: jax.Array,
    A_w_uv: jax.Array,
    A_w_o: jax.Array,
    B_x: jax.Array,
    B_w_r: jax.Array,
    B_w_gate: jax.Array,
    B_w_up: jax.Array,
    B_w_down: jax.Array,
):
    del B_x
    return _forward(A_x, A_c_kv, A_w_q, A_w_uk, A_w_uv, A_w_o, B_w_r, B_w_gate, B_w_up, B_w_down)
```

```python
import functools

import jax
import jax.numpy as jnp
from jax import lax
import jax.experimental.pallas as pl
import jax.experimental.pallas.tpu as pltpu

_F32 = jnp.float32
_BF16 = jnp.bfloat16
_LANES = 128
_BLOCK = 64
_PERIOD = 4 * _BLOCK
_PATTERN = ((((192, 248),), ((248, 256), (128, 192))),
            (((0, 56),), ((56, 64), (64, 128))))
_NT = (((1,), (1,)), ((), ()))


def _layernorm(v):
    mean = jnp.mean(v, axis=-1, keepdims=True)
    cen = v - mean
    var = jnp.mean(cen * cen, axis=-1, keepdims=True)
    return cen / jnp.sqrt(var + 1e-5)


def _kernel(x_hbm, ckv_hbm, wq_hbm, wuk_hbm, wuv_hbm, wo_hbm, wr_hbm, wg_hbm, wu_hbm, wd_hbm,
            o_ref,
            x_v, wr_v, ckv_v, wq_v, wuk_v, wuv_v, wo_v, wg_v, wu_v, wd_v,
            tbl_ref, perm_ref, z_ref, s_ref, acc_ref, ctx_ref, act_ref, sems, small_sems,
            *, depth, shifts, ramp=3, late_tiles=4, late_keys=3, down_edges=(4, 8)):
    M, H, D = wq_v.shape
    Sk, Dc = ckv_v.shape
    G = _LANES // H
    T = Dc // G
    F = wg_v.shape[0]
    rows = _LANES
    tiles = 16
    f_full, f_rest = F // rows, F % rows

    runs, first = [], [0]

    def add_run(window, steps, repeat=1):
        if repeat > 0:
            runs.append((window, steps))
            first.append(first[-1] + repeat * len(steps))

    def add_array(src, dst, shift, ramp=0):
        length, total = src.shape[0], src.size * 2 // 1024

        def window(base):
            def at(period, lo, hi):
                start = (base + lo) * length // total + period * (_PERIOD * length // total)
                if not isinstance(start, int) and length == total:
                    start = pl.multiple_of(start, 8)
                index = pl.ds(start, (hi - lo) * length // total)
                return src.at[index], dst.at[index]
            return at

        def add_period(j, repeat=1, extra=()):
            base = j * _PERIOD - shift
            steps = [[[(max(lo, -base), min(hi, total - base)) for lo, hi in part] for part in step]
                     for step in _PATTERN]
            steps[-1][-1] += extra
            add_run(window(base), steps, repeat)

        periods = (total + shift + _PERIOD // 2) // _PERIOD
        left = total + shift - periods * _PERIOD
        if ramp:
            edges = [0] + list(range(_BLOCK + -shift % _BLOCK, ramp * _PERIOD - shift + 1, _BLOCK))
            for piece in zip(edges[:-1], edges[1:]):
                add_run(lambda period, lo, hi: window(0)(0, lo, hi), [[[], [piece]]])
        else:
            add_period(0)
        begin = max(ramp, 1)
        origin = first[-1] - begin * len(_PATTERN)
        add_period(begin, periods - 1 - begin)
        add_period(periods - 1, extra=[(_PERIOD + lo, _PERIOD + min(lo + _BLOCK, left))
                                       for lo in range(0, left, _BLOCK)])

        def ready(n):
            j = min(max(pl.cdiv(n * total // length + shift, _PERIOD), begin), periods)
            return origin + j * len(_PATTERN) - 1
        return ready

    wq_ready = add_array(wq_hbm, wq_v, shifts[0], ramp=ramp)
    wuk_ready = add_array(wuk_hbm, wuk_v, shifts[1])
    ckv_ready = add_array(ckv_hbm, ckv_v, shifts[2])
    wuv_ready = add_array(wuv_hbm, wuv_v, shifts[3])
    wo_ready = add_array(wo_hbm, wo_v, shifts[4])
    add_array(wg_hbm, wg_v, shifts[5])
    wu_ready = add_array(wu_hbm, wu_v, shifts[6])
    wd_ready = add_array(wd_hbm, wd_v, shifts[7])
    n_steps = first[-1]

    def kind(step):
        if step >= n_steps:
            return None
        k = max(k for k in range(len(runs)) if first[k] <= step)
        return k, (step - first[k]) % len(runs[k][1])

    def copies(step, i, k, phase):
        window, steps = runs[k]
        period = (step - first[k]) // len(steps) + i
        sem = (2 * step + 4 * i) & (sems.shape[0] - 1)
        return [[pltpu.make_async_copy(*window(period, lo, hi), sems.at[sem + queue])
                 for lo, hi in part if lo < hi] for queue, part in enumerate(steps[phase])]

    def start_step(step, i, k, phase):
        for queue, part in enumerate(copies(step, i, k, phase)):
            for copy in part:
                copy.start(priority=queue)

    def tick(step, i, landed, ahead):
        early, late = copies(step, i, *landed) if landed else ((), ())
        for copy in late:
            copy.wait()
        if ahead:
            start_step(step + depth, i, *ahead)
        for copy in early:
            copy.wait()

    now = [0]

    def pairs(n, body=None, carry=None):
        lo = now[0]
        now[0] += 2 * n

        def kinds(i):
            return [(kind(g), kind(g + depth)) for g in (lo + 2 * i, lo + 2 * i + 1)]

        a = 0
        while a < n:
            b = a + 1
            while b < n and kinds(b) == kinds(a):
                b += 1

            def step(i, c, ks=kinds(a)):
                tick(lo, i, *ks[0])
                next_tick = functools.partial(tick, lo + 1, i, *ks[1])
                return next_tick() if body is None else body(i, c, next_tick)

            carry = step(a, carry) if b - a == 1 else lax.fori_loop(a, b, step, carry)
            a = b
        return carry

    def idle(n):
        if n > 0:
            pairs(n // 2)
            if n % 2:
                tick(now[0], 0, kind(now[0]), kind(now[0] + depth))
                now[0] += 1

    def stream(n, body, carry, ready):
        idle(max(ready(i) - 2 * i for i in range(n)) - now[0])
        return pairs(n, body, carry)

    def aligned(start, size):
        return pl.ds(start if isinstance(start, int) else pl.multiple_of(start, size), size)

    x_copy = pltpu.make_async_copy(x_hbm, x_v, small_sems.at[0])
    wr_copy = pltpu.make_async_copy(wr_hbm, wr_v, small_sems.at[1])
    x_copy.start()
    for g in range(depth):
        start_step(g, 0, *kind(g))
    wr_copy.start()

    x_copy.wait()
    x = x_v[0].astype(_F32)
    xn = _layernorm(x).astype(_BF16).astype(_F32)
    for j in range(M // _LANES):
        blk = jnp.broadcast_to(xn[:, j * _LANES:(j + 1) * _LANES], (_LANES, _LANES))
        tbl_ref[j * _LANES:(j + 1) * _LANES, :] = blk.T

    for j in range(G):
        idle(1)
        source = lax.broadcasted_iota(jnp.int32, (T, Dc), 0) * G + j
        hit = source == lax.broadcasted_iota(jnp.int32, (T, Dc), 1)
        perm_ref[j * T:(j + 1) * T, :] = jnp.where(hit, 1.0, 0.0).astype(_BF16)

    def q_body(i, acc, next_tick):
        for b in range(tiles // 2):
            if b == tiles // 4:
                next_tick()
            base = pl.multiple_of(i * tiles * G + b * 8, 8)
            xb = tbl_ref[pl.ds(base, 8), :]
            for k in range(8):
                acc = acc + wq_v[base + k].astype(_F32) * xb[k:k + 1, :]
        return acc

    q = stream(M // (tiles * G), q_body, jnp.zeros((H, D), _F32),
               lambda i: wq_ready((i + 1) * tiles * G)).astype(_BF16)

    own_head = (lax.broadcasted_iota(jnp.int32, (H, G * H), 1) % H
                == lax.broadcasted_iota(jnp.int32, (H, G * H), 0))

    def uk_body(i, carry, next_tick):
        full = []
        for k in range(8):
            if k == 4:
                next_tick()
            w = wuk_v[pl.ds((8 * i + k) * G, G)].reshape(G * H, D)
            full.append(lax.dot_general(q, w, _NT, preferred_element_type=_F32))
        z_ref[aligned(i * 8, 8), :] = jnp.concatenate(
            [jnp.sum(jnp.where(own_head, f, 0.0), axis=0, keepdims=True) for f in full], axis=0)
        return carry

    stream(T // 8, uk_body, 0, lambda i: wuk_ready((i + 1) * 8 * G))
    idle(1)
    zt = z_ref[...].T * (D ** -0.5)
    qa = jnp.concatenate([zt[j * H:(j + 1) * H, :] for j in range(G)], axis=1).astype(_BF16)
    idle(1)
    qa = jnp.dot(qa, perm_ref[...], preferred_element_type=_F32).astype(_BF16)

    def score_body(i, peak, next_tick):
        for k in range(2):
            if k == 1:
                next_tick()
            s = lax.dot_general(qa, ckv_v[aligned((2 * i + k) * rows, rows), :], _NT,
                                preferred_element_type=_F32)
            s_ref[2 * i + k] = s
            peak = jnp.maximum(peak, s)
        return peak

    peak = stream(Sk // (2 * rows), score_body, jnp.full((H, rows), -jnp.inf, _F32),
                  lambda i: ckv_ready((i + 1) * 2 * rows))
    peak = jnp.broadcast_to(jnp.max(peak, axis=-1, keepdims=True), (H, rows))

    def value_body(i, total, next_tick):
        acc = acc_ref[...]
        for k in range(4):
            if k == late_keys:
                next_tick()
            p = jnp.exp(s_ref[4 * i + k] - peak)
            total = total + p
            acc = acc + jnp.dot(p.astype(_BF16), ckv_v[aligned((4 * i + k) * rows, rows), :],
                                preferred_element_type=_F32)
        acc_ref[...] = acc
        return total

    acc_ref[...] = jnp.zeros_like(acc_ref)
    total = pairs(Sk // (4 * rows), value_body, jnp.zeros((H, rows), _F32))
    idle(1)
    lat = acc_ref[...] / jnp.sum(total, axis=-1, keepdims=True)
    z_ref[...] = jnp.concatenate([lat[:, j * T:(j + 1) * T] for j in range(G)], axis=0).T

    def uv_body(i, ctx, next_tick):
        zb = z_ref[aligned(i * tiles, tiles), :]
        for k in range(tiles):
            if k == tiles - late_tiles:
                next_tick()
            lhs = jnp.where(own_head, zb[k:k + 1, :], 0.0).astype(_BF16)
            t = i * tiles + k
            w = jnp.concatenate([wuv_v[j * T + t] for j in range(G)], axis=0)
            ctx = ctx + jnp.dot(lhs, w, preferred_element_type=_F32)
        return ctx

    ctx_ref[...] = stream(T // tiles, uv_body, jnp.zeros((H, D), _F32), lambda i: wuv_ready(Dc))

    heads = tiles * _LANES // M

    def o_body(i, carry, next_tick):
        for k in range(heads):
            if k == heads - 1:
                next_tick()
            lhs = jnp.broadcast_to(ctx_ref[pl.ds(heads * i + k, 1), :], (8, D)).astype(_BF16)
            w = wo_v[aligned((heads * i + k) * D, D), :]
            carry = carry + jnp.dot(lhs, w, preferred_element_type=_F32)
        return carry

    attn = stream(H // heads, o_body, jnp.zeros((8, M), _F32),
                  lambda i: wo_ready((i + 1) * heads * D))

    idle(1)
    h = x + attn[0:1, :]
    hn = _layernorm(h)
    hb = jnp.broadcast_to(hn, (8, M)).astype(_BF16)
    idle(1)
    wr_copy.wait()
    wr = wr_v[...].astype(_F32)
    r = sum(jnp.sum(hn[:, j * _LANES:(j + 1) * _LANES] * wr[j:j + 1, :], axis=-1, keepdims=True)
            for j in range(M // _LANES))
    gate = jax.nn.sigmoid(r)
    resid = h + (hn + hn * 0.0)

    def project(w_v, window):
        return lax.dot_general(hb, w_v[window, :], _NT, preferred_element_type=_F32)

    def silu(v):
        return v * jax.nn.sigmoid(v)

    def up_body(i, carry, next_tick):
        g = silu(project(wg_v, aligned(2 * i * rows, 2 * rows)))
        u0 = project(wu_v, aligned(2 * i * rows, rows))
        next_tick()
        u1 = project(wu_v, aligned((2 * i + 1) * rows, rows))
        act_ref[2 * i] = g[:, :rows] * u0
        act_ref[2 * i + 1] = g[:, rows:] * u1
        return carry

    stream(f_full // 2, up_body, 0, lambda i: wu_ready((i + 1) * 2 * rows))
    idle(wu_ready(F) + 1 - now[0])
    rest = pl.ds(f_full * rows, f_rest)
    act_rest = (silu(project(wg_v, rest)) * project(wu_v, rest)).astype(_BF16)
    y = jnp.zeros((8, M), _F32)
    done = 0
    for edge in down_edges + (f_full + 1,):
        idle(wd_ready(min(edge * rows, F)) + 1 - now[0])
        for i in range(done, edge):
            act, window = ((act_ref[i].astype(_BF16), pl.ds(i * rows, rows)) if i < f_full
                           else (act_rest, rest))
            y = y + jnp.dot(act, wd_v[window, :], preferred_element_type=_F32)
        done = edge
    assert now[0] >= n_steps and f_full % 2 == 0
    o_ref[0] = (resid + y[0:1, :] * gate).astype(o_ref.dtype)


def _forward(A_x, A_c_kv, A_w_q, A_w_uk, A_w_uv, A_w_o, B_w_r, B_w_gate, B_w_up, B_w_down, *,
             depth=12, shifts=(32,) * 6 + (64, 96), params=None, **debug):
    B, Sq, M = A_x.shape
    _, Sk, Dc = A_c_kv.shape
    _, H, D = A_w_q.shape
    F = B_w_gate.shape[1]
    assert B == 1 and Sq == 1 and D == _LANES and _LANES % H == 0 and Dc == M
    G = _LANES // H
    T = Dc // G
    rows = _LANES
    assert T == _LANES

    hbm = pl.BlockSpec(memory_space=pltpu.HBM)
    return pl.pallas_call(
        functools.partial(_kernel, depth=depth, shifts=shifts, **debug),
        out_shape=jax.ShapeDtypeStruct((B, Sq, M), A_x.dtype),
        in_specs=[hbm] * 10,
        out_specs=pl.BlockSpec(memory_space=pltpu.VMEM),
        scratch_shapes=[
            pltpu.VMEM((B, Sq, M), _BF16),
            pltpu.VMEM((M // _LANES, _LANES), _BF16),
            pltpu.VMEM((Sk, Dc), _BF16),
            pltpu.VMEM((M, H, D), _BF16),
            pltpu.VMEM((Dc, H, D), _BF16),
            pltpu.VMEM((Dc, H, D), _BF16),
            pltpu.VMEM((H * D, M), _BF16),
            pltpu.VMEM((F, M), _BF16),
            pltpu.VMEM((F, M), _BF16),
            pltpu.VMEM((F, M), _BF16),
            pltpu.VMEM((M, _LANES), _F32),
            pltpu.VMEM((Dc, Dc), _BF16),
            pltpu.VMEM((T, G * H), _F32),
            pltpu.VMEM((Sk // rows, H, rows), _F32),
            pltpu.VMEM((H, Dc), _F32),
            pltpu.VMEM((H, D), _F32),
            pltpu.VMEM((F // rows, 8, rows), _F32),
            pltpu.SemaphoreType.DMA((2 * pl.next_power_of_2(depth + 1),)),
            pltpu.SemaphoreType.DMA((2,)),
        ],
        compiler_params=pltpu.CompilerParams(vmem_limit_bytes=64 * 2**20, **(params or dict(disable_semaphore_checks=True, disable_bounds_checks=True))),
    )(
        A_x,
        A_c_kv.reshape(Sk, Dc),
        A_w_q,
        A_w_uk,
        A_w_uv,
        A_w_o.reshape(H * D, M),
        B_w_r.reshape(M // _LANES, _LANES),
        B_w_gate.T,
        B_w_up.T,
        B_w_down,
    )


@jax.jit
def pallas_sequential_preLN__compressed_kv_cla__moe_arch_mod__decode_kernel(
    A_x: jax.Array,
    A_c_kv: jax.Array,
    A_w_q: jax.Array,
    A_w_uk: jax.Array,
    A_w_uv: jax.Array,
    A_w_o: jax.Array,
    B_x: jax.Array,
    B_w_r: jax.Array,
    B_w_gate: jax.Array,
    B_w_up: jax.Array,
    B_w_down: jax.Array,
):
    del B_x
    return _forward(A_x, A_c_kv, A_w_q, A_w_uk, A_w_uv, A_w_o, B_w_r, B_w_gate, B_w_up, B_w_down)
```

```python
import functools

import jax
import jax.numpy as jnp
from jax import lax
import jax.experimental.pallas as pl
import jax.experimental.pallas.tpu as pltpu

_F32 = jnp.float32
_BF16 = jnp.bfloat16
_LANES = 128
_BLOCK = 64
_PERIOD = 4 * _BLOCK
_NT = (((1,), (1,)), ((), ()))


def _layernorm(v):
    mean = jnp.mean(v, axis=-1, keepdims=True)
    cen = v - mean
    var = jnp.mean(cen * cen, axis=-1, keepdims=True)
    return cen / jnp.sqrt(var + 1e-5)


def _kernel(x_hbm, ckv_hbm, wq_hbm, wuk_hbm, wuv_hbm, wo_hbm, wr_hbm, wg_hbm, wu_hbm, wd_hbm,
            o_ref,
            x_v, wr_v, ckv_v, wq_v, wuk_v, wuv_v, wo_v, wg_v, wu_v, wd_v,
            tbl_ref, perm_ref, z_ref, s_ref, acc_ref, ctx_ref, act_ref, sems, small_sems,
            *, depth, shifts, order=((2, 3), (0, 1)), head=56, ramp=3, late_tiles=4, late_keys=3, down_edges=(4, 8)):
    M, H, D = wq_v.shape
    Sk, Dc = ckv_v.shape
    G = _LANES // H
    T = Dc // G
    F = wg_v.shape[0]
    rows = _LANES
    tiles = 16
    f_full, f_rest = F // rows, F % rows

    runs, first = [], [0]
    pattern = [(((a * _BLOCK, a * _BLOCK + head),),
                ((a * _BLOCK + head, (a + 1) * _BLOCK), (b * _BLOCK, (b + 1) * _BLOCK)))
               for a, b in order]

    def add_run(window, steps, repeat=1):
        if repeat > 0:
            runs.append((window, steps))
            first.append(first[-1] + repeat * len(steps))

    def add_array(src, dst, shift, ramp=0):
        length, total = src.shape[0], src.size * 2 // 1024

        def window(base):
            def at(period, lo, hi):
                start = (base + lo) * length // total + period * (_PERIOD * length // total)
                if not isinstance(start, int) and length == total:
                    start = pl.multiple_of(start, 8)
                index = pl.ds(start, (hi - lo) * length // total)
                return src.at[index], dst.at[index]
            return at

        def add_period(j, repeat=1, extra=()):
            base = j * _PERIOD - shift
            steps = [[[(max(lo, -base), min(hi, total - base)) for lo, hi in part] for part in step]
                     for step in pattern]
            steps[-1][-1] += extra
            add_run(window(base), steps, repeat)

        periods = (total + shift + _PERIOD // 2) // _PERIOD
        left = total + shift - periods * _PERIOD
        if ramp:
            edges = [0] + list(range(_BLOCK + -shift % _BLOCK, ramp * _PERIOD - shift + 1, _BLOCK))
            for piece in zip(edges[:-1], edges[1:]):
                add_run(lambda period, lo, hi: window(0)(0, lo, hi), [[[], [piece]]])
        else:
            add_period(0)
        begin = max(ramp, 1)
        origin = first[-1] - begin * len(pattern)
        add_period(begin, periods - 1 - begin)
        add_period(periods - 1, extra=[(_PERIOD + lo, _PERIOD + min(lo + _BLOCK, left))
                                       for lo in range(0, left, _BLOCK)])

        def ready(n):
            j = min(max(pl.cdiv(n * total // length + shift, _PERIOD), begin), periods)
            return origin + j * len(pattern) - 1
        return ready

    wq_ready = add_array(wq_hbm, wq_v, shifts[0], ramp=ramp)
    wuk_ready = add_array(wuk_hbm, wuk_v, shifts[1])
    ckv_ready = add_array(ckv_hbm, ckv_v, shifts[2])
    wuv_ready = add_array(wuv_hbm, wuv_v, shifts[3])
    wo_ready = add_array(wo_hbm, wo_v, shifts[4])
    add_array(wg_hbm, wg_v, shifts[5])
    wu_ready = add_array(wu_hbm, wu_v, shifts[6])
    wd_ready = add_array(wd_hbm, wd_v, shifts[7])
    n_steps = first[-1]

    def kind(step):
        if step >= n_steps:
            return None
        k = max(k for k in range(len(runs)) if first[k] <= step)
        return k, (step - first[k]) % len(runs[k][1])

    def copies(step, i, k, phase):
        window, steps = runs[k]
        period = (step - first[k]) // len(steps) + i
        sem = (2 * step + 4 * i) & (sems.shape[0] - 1)
        return [[pltpu.make_async_copy(*window(period, lo, hi), sems.at[sem + queue])
                 for lo, hi in part if lo < hi] for queue, part in enumerate(steps[phase])]

    def start_step(step, i, k, phase):
        for queue, part in enumerate(copies(step, i, k, phase)):
            for copy in part:
                copy.start(priority=queue)

    def tick(step, i, landed, ahead):
        early, late = copies(step, i, *landed) if landed else ((), ())
        for copy in late:
            copy.wait()
        if ahead:
            start_step(step + depth, i, *ahead)
        for copy in early:
            copy.wait()

    now = [0]

    def pairs(n, body=None, carry=None):
        lo = now[0]
        now[0] += 2 * n

        def kinds(i):
            return [(kind(g), kind(g + depth)) for g in (lo + 2 * i, lo + 2 * i + 1)]

        a = 0
        while a < n:
            b = a + 1
            while b < n and kinds(b) == kinds(a):
                b += 1

            def step(i, c, ks=kinds(a)):
                tick(lo, i, *ks[0])
                next_tick = functools.partial(tick, lo + 1, i, *ks[1])
                return next_tick() if body is None else body(i, c, next_tick)

            carry = step(a, carry) if b - a == 1 else lax.fori_loop(a, b, step, carry)
            a = b
        return carry

    def idle(n):
        if n > 0:
            pairs(n // 2)
            if n % 2:
                tick(now[0], 0, kind(now[0]), kind(now[0] + depth))
                now[0] += 1

    def stream(n, body, carry, ready):
        idle(max(ready(i) - 2 * i for i in range(n)) - now[0])
        return pairs(n, body, carry)

    def aligned(start, size):
        return pl.ds(start if isinstance(start, int) else pl.multiple_of(start, size), size)

    x_copy = pltpu.make_async_copy(x_hbm, x_v, small_sems.at[0])
    wr_copy = pltpu.make_async_copy(wr_hbm, wr_v, small_sems.at[1])
    x_copy.start()
    for g in range(depth):
        start_step(g, 0, *kind(g))
    wr_copy.start()

    x_copy.wait()
    x = x_v[0].astype(_F32)
    xn = _layernorm(x).astype(_BF16).astype(_F32)
    for j in range(M // _LANES):
        blk = jnp.broadcast_to(xn[:, j * _LANES:(j + 1) * _LANES], (_LANES, _LANES))
        tbl_ref[j * _LANES:(j + 1) * _LANES, :] = blk.T

    for j in range(G):
        idle(1)
        source = lax.broadcasted_iota(jnp.int32, (T, Dc), 0) * G + j
        hit = source == lax.broadcasted_iota(jnp.int32, (T, Dc), 1)
        perm_ref[j * T:(j + 1) * T, :] = jnp.where(hit, 1.0, 0.0).astype(_BF16)

    def q_body(i, acc, next_tick):
        for b in range(tiles // 2):
            if b == tiles // 4:
                next_tick()
            base = pl.multiple_of(i * tiles * G + b * 8, 8)
            xb = tbl_ref[pl.ds(base, 8), :]
            for k in range(8):
                acc = acc + wq_v[base + k].astype(_F32) * xb[k:k + 1, :]
        return acc

    q = stream(M // (tiles * G), q_body, jnp.zeros((H, D), _F32),
               lambda i: wq_ready((i + 1) * tiles * G)).astype(_BF16)

    own_head = (lax.broadcasted_iota(jnp.int32, (H, G * H), 1) % H
                == lax.broadcasted_iota(jnp.int32, (H, G * H), 0))

    def uk_body(i, carry, next_tick):
        full = []
        for k in range(8):
            if k == 4:
                next_tick()
            w = wuk_v[pl.ds((8 * i + k) * G, G)].reshape(G * H, D)
            full.append(lax.dot_general(q, w, _NT, preferred_element_type=_F32))
        z_ref[aligned(i * 8, 8), :] = jnp.concatenate(
            [jnp.sum(jnp.where(own_head, f, 0.0), axis=0, keepdims=True) for f in full], axis=0)
        return carry

    stream(T // 8, uk_body, 0, lambda i: wuk_ready((i + 1) * 8 * G))
    idle(1)
    zt = z_ref[...].T * (D ** -0.5)
    qa = jnp.concatenate([zt[j * H:(j + 1) * H, :] for j in range(G)], axis=1).astype(_BF16)
    idle(1)
    qa = jnp.dot(qa, perm_ref[...], preferred_element_type=_F32).astype(_BF16)

    def score_body(i, peak, next_tick):
        for k in range(2):
            if k == 1:
                next_tick()
            s = lax.dot_general(qa, ckv_v[aligned((2 * i + k) * rows, rows), :], _NT,
                                preferred_element_type=_F32)
            s_ref[2 * i + k] = s
            peak = jnp.maximum(peak, s)
        return peak

    peak = stream(Sk // (2 * rows), score_body, jnp.full((H, rows), -jnp.inf, _F32),
                  lambda i: ckv_ready((i + 1) * 2 * rows))
    peak = jnp.broadcast_to(jnp.max(peak, axis=-1, keepdims=True), (H, rows))

    def value_body(i, total, next_tick):
        acc = acc_ref[...]
        for k in range(4):
            if k == late_keys:
                next_tick()
            p = jnp.exp(s_ref[4 * i + k] - peak)
            total = total + p
            acc = acc + jnp.dot(p.astype(_BF16), ckv_v[aligned((4 * i + k) * rows, rows), :],
                                preferred_element_type=_F32)
        acc_ref[...] = acc
        return total

    acc_ref[...] = jnp.zeros_like(acc_ref)
    total = pairs(Sk // (4 * rows), value_body, jnp.zeros((H, rows), _F32))
    idle(1)
    lat = acc_ref[...] / jnp.sum(total, axis=-1, keepdims=True)
    z_ref[...] = jnp.concatenate([lat[:, j * T:(j + 1) * T] for j in range(G)], axis=0).T

    def uv_body(i, ctx, next_tick):
        zb = z_ref[aligned(i * tiles, tiles), :]
        for k in range(tiles):
            if k == tiles - late_tiles:
                next_tick()
            lhs = jnp.where(own_head, zb[k:k + 1, :], 0.0).astype(_BF16)
            t = i * tiles + k
            w = jnp.concatenate([wuv_v[j * T + t] for j in range(G)], axis=0)
            ctx = ctx + jnp.dot(lhs, w, preferred_element_type=_F32)
        return ctx

    ctx_ref[...] = stream(T // tiles, uv_body, jnp.zeros((H, D), _F32), lambda i: wuv_ready(Dc))

    heads = tiles * _LANES // M

    def o_body(i, carry, next_tick):
        for k in range(heads):
            if k == heads - 1:
                next_tick()
            lhs = jnp.broadcast_to(ctx_ref[pl.ds(heads * i + k, 1), :], (8, D)).astype(_BF16)
            w = wo_v[aligned((heads * i + k) * D, D), :]
            carry = carry + jnp.dot(lhs, w, preferred_element_type=_F32)
        return carry

    attn = stream(H // heads, o_body, jnp.zeros((8, M), _F32),
                  lambda i: wo_ready((i + 1) * heads * D))

    idle(1)
    h = x + attn[0:1, :]
    hn = _layernorm(h)
    hb = jnp.broadcast_to(hn, (8, M)).astype(_BF16)
    idle(1)
    wr_copy.wait()
    wr = wr_v[...].astype(_F32)
    r = sum(jnp.sum(hn[:, j * _LANES:(j + 1) * _LANES] * wr[j:j + 1, :], axis=-1, keepdims=True)
            for j in range(M // _LANES))
    gate = jax.nn.sigmoid(r)
    resid = h + (hn + hn * 0.0)

    def project(w_v, window):
        return lax.dot_general(hb, w_v[window, :], _NT, preferred_element_type=_F32)

    def silu(v):
        return v * jax.nn.sigmoid(v)

    def up_body(i, carry, next_tick):
        g = silu(project(wg_v, aligned(2 * i * rows, 2 * rows)))
        u0 = project(wu_v, aligned(2 * i * rows, rows))
        next_tick()
        u1 = project(wu_v, aligned((2 * i + 1) * rows, rows))
        act_ref[2 * i] = g[:, :rows] * u0
        act_ref[2 * i + 1] = g[:, rows:] * u1
        return carry

    stream(f_full // 2, up_body, 0, lambda i: wu_ready((i + 1) * 2 * rows))
    idle(wu_ready(F) + 1 - now[0])
    rest = pl.ds(f_full * rows, f_rest)
    act_rest = (silu(project(wg_v, rest)) * project(wu_v, rest)).astype(_BF16)
    y = jnp.zeros((8, M), _F32)
    done = 0
    for edge in down_edges + (f_full + 1,):
        idle(wd_ready(min(edge * rows, F)) + 1 - now[0])
        for i in range(done, edge):
            act, window = ((act_ref[i].astype(_BF16), pl.ds(i * rows, rows)) if i < f_full
                           else (act_rest, rest))
            y = y + jnp.dot(act, wd_v[window, :], preferred_element_type=_F32)
        done = edge
    assert now[0] >= n_steps and f_full % 2 == 0
    o_ref[0] = (resid + y[0:1, :] * gate).astype(o_ref.dtype)


def _forward(A_x, A_c_kv, A_w_q, A_w_uk, A_w_uv, A_w_o, B_w_r, B_w_gate, B_w_up, B_w_down, *,
             depth=12, shifts=(32,) * 6 + (128, 224), params=None, **debug):
    B, Sq, M = A_x.shape
    _, Sk, Dc = A_c_kv.shape
    _, H, D = A_w_q.shape
    F = B_w_gate.shape[1]
    assert B == 1 and Sq == 1 and D == _LANES and _LANES % H == 0 and Dc == M
    G = _LANES // H
    T = Dc // G
    rows = _LANES
    assert T == _LANES

    hbm = pl.BlockSpec(memory_space=pltpu.HBM)
    return pl.pallas_call(
        functools.partial(_kernel, depth=depth, shifts=shifts, **debug),
        out_shape=jax.ShapeDtypeStruct((B, Sq, M), A_x.dtype),
        in_specs=[hbm] * 10,
        out_specs=pl.BlockSpec(memory_space=pltpu.VMEM),
        scratch_shapes=[
            pltpu.VMEM((B, Sq, M), _BF16),
            pltpu.VMEM((M // _LANES, _LANES), _BF16),
            pltpu.VMEM((Sk, Dc), _BF16),
            pltpu.VMEM((M, H, D), _BF16),
            pltpu.VMEM((Dc, H, D), _BF16),
            pltpu.VMEM((Dc, H, D), _BF16),
            pltpu.VMEM((H * D, M), _BF16),
            pltpu.VMEM((F, M), _BF16),
            pltpu.VMEM((F, M), _BF16),
            pltpu.VMEM((F, M), _BF16),
            pltpu.VMEM((M, _LANES), _F32),
            pltpu.VMEM((Dc, Dc), _BF16),
            pltpu.VMEM((T, G * H), _F32),
            pltpu.VMEM((Sk // rows, H, rows), _F32),
            pltpu.VMEM((H, Dc), _F32),
            pltpu.VMEM((H, D), _F32),
            pltpu.VMEM((F // rows, 8, rows), _F32),
            pltpu.SemaphoreType.DMA((2 * pl.next_power_of_2(depth + 1),)),
            pltpu.SemaphoreType.DMA((2,)),
        ],
        compiler_params=pltpu.CompilerParams(vmem_limit_bytes=64 * 2**20, **(params or dict(disable_semaphore_checks=True, disable_bounds_checks=True))),
    )(
        A_x,
        A_c_kv.reshape(Sk, Dc),
        A_w_q,
        A_w_uk,
        A_w_uv,
        A_w_o.reshape(H * D, M),
        B_w_r.reshape(M // _LANES, _LANES),
        B_w_gate.T,
        B_w_up.T,
        B_w_down,
    )


@jax.jit
def pallas_sequential_preLN__compressed_kv_cla__moe_arch_mod__decode_kernel(
    A_x: jax.Array,
    A_c_kv: jax.Array,
    A_w_q: jax.Array,
    A_w_uk: jax.Array,
    A_w_uv: jax.Array,
    A_w_o: jax.Array,
    B_x: jax.Array,
    B_w_r: jax.Array,
    B_w_gate: jax.Array,
    B_w_up: jax.Array,
    B_w_down: jax.Array,
):
    del B_x
    return _forward(A_x, A_c_kv, A_w_q, A_w_uk, A_w_uv, A_w_o, B_w_r, B_w_gate, B_w_up, B_w_down)
```

```python
import functools

import jax
import jax.numpy as jnp
from jax import lax
import jax.experimental.pallas as pl
import jax.experimental.pallas.tpu as pltpu

_F32 = jnp.float32
_BF16 = jnp.bfloat16
_LANES = 128
_BLOCK = 64
_PERIOD = 4 * _BLOCK
_HEAD = 56
_PATTERN = tuple((((a * _BLOCK, a * _BLOCK + _HEAD),),
                  ((b * _BLOCK, (b + 1) * _BLOCK), (a * _BLOCK + _HEAD, (a + 1) * _BLOCK)))
                 for a, b in ((1, 3), (2, 0)))
_SHIFT = 32
_DEPTH = 12
_RAMP = 3
_NT = (((1,), (1,)), ((), ()))


def _layernorm(v):
    mean = jnp.mean(v, axis=-1, keepdims=True)
    cen = v - mean
    var = jnp.mean(cen * cen, axis=-1, keepdims=True)
    return cen / jnp.sqrt(var + 1e-5)


def _kernel(x_hbm, ckv_hbm, wq_hbm, wuk_hbm, wuv_hbm, wo_hbm, wr_hbm, wg_hbm, wu_hbm, wd_hbm,
            o_ref,
            x_v, wr_v, ckv_v, wq_v, wuk_v, wuv_v, wo_v, wg_v, wu_v, wd_v,
            tbl_ref, perm_ref, z_ref, s_ref, acc_ref, ctx_ref, act_ref, sems, small_sems):
    M, H, D = wq_v.shape
    Sk, Dc = ckv_v.shape
    G = _LANES // H
    T = Dc // G
    F = wg_v.shape[0]
    rows = _LANES
    tiles = 16
    f_full, f_rest = F // rows, F % rows

    runs, first, queued = [], [0], [0]

    def add_run(window, steps, repeat=1):
        if repeat > 0:
            runs.append((window, steps))
            first.append(first[-1] + repeat * len(steps))

    def add_array(src, dst, ramp=0):
        length, total = src.shape[0], src.size * 2 // 1024
        shift = (_SHIFT + queued[0]) % _PERIOD
        queued[0] += total

        def window(base):
            def at(period, lo, hi):
                start = (base + lo) * length // total + period * (_PERIOD * length // total)
                if not isinstance(start, int) and length == total:
                    start = pl.multiple_of(start, 8)
                index = pl.ds(start, (hi - lo) * length // total)
                return src.at[index], dst.at[index]
            return at

        def add_period(j, repeat=1, extra=()):
            base = j * _PERIOD - shift
            steps = [[[(max(lo, -base), min(hi, total - base)) for lo, hi in part] for part in step]
                     for step in _PATTERN]
            steps[-1][-1] += extra
            add_run(window(base), steps, repeat)

        periods = (total + shift + _PERIOD // 2) // _PERIOD
        left = total + shift - periods * _PERIOD
        if ramp:
            edges = [0] + list(range(_BLOCK + -shift % _BLOCK, ramp * _PERIOD - shift + 1, _BLOCK))
            for piece in zip(edges[:-1], edges[1:]):
                add_run(lambda period, lo, hi: window(0)(0, lo, hi), [[[], [piece]]])
        else:
            add_period(0)
        begin = max(ramp, 1)
        origin = first[-1] - begin * len(_PATTERN)
        add_period(begin, periods - 1 - begin)
        add_period(periods - 1, extra=[(_PERIOD + lo, _PERIOD + min(lo + _BLOCK, left))
                                       for lo in range(0, left, _BLOCK)])

        def ready(n):
            j = min(max(pl.cdiv(n * total // length + shift, _PERIOD), begin), periods)
            return origin + j * len(_PATTERN) - 1
        return ready

    wq_ready = add_array(wq_hbm, wq_v, ramp=_RAMP)
    wuk_ready = add_array(wuk_hbm, wuk_v)
    ckv_ready = add_array(ckv_hbm, ckv_v)
    wuv_ready = add_array(wuv_hbm, wuv_v)
    wo_ready = add_array(wo_hbm, wo_v)
    add_array(wg_hbm, wg_v)
    wu_ready = add_array(wu_hbm, wu_v)
    wd_ready = add_array(wd_hbm, wd_v)
    n_steps = first[-1]

    def kind(step):
        if step >= n_steps:
            return None
        k = max(k for k in range(len(runs)) if first[k] <= step)
        return k, (step - first[k]) % len(runs[k][1])

    def copies(step, i, k, phase):
        window, steps = runs[k]
        period = (step - first[k]) // len(steps) + i
        sem = (2 * step + 4 * i) & (sems.shape[0] - 1)
        return [[pltpu.make_async_copy(*window(period, lo, hi), sems.at[sem + queue])
                 for lo, hi in part if lo < hi] for queue, part in enumerate(steps[phase])]

    def start_step(step, i, k, phase):
        for queue, part in enumerate(copies(step, i, k, phase)):
            for copy in part:
                copy.start(priority=queue)

    def tick(step, i, landed, ahead):
        early, late = copies(step, i, *landed) if landed else ((), ())
        for copy in late:
            copy.wait()
        if ahead:
            start_step(step + _DEPTH, i, *ahead)
        for copy in early:
            copy.wait()

    now = [0]

    def pairs(n, body=None, carry=None):
        lo = now[0]
        now[0] += 2 * n

        def kinds(i):
            return [(kind(g), kind(g + _DEPTH)) for g in (lo + 2 * i, lo + 2 * i + 1)]

        a = 0
        while a < n:
            b = a + 1
            while b < n and kinds(b) == kinds(a):
                b += 1

            def step(i, c, ks=kinds(a)):
                tick(lo, i, *ks[0])
                next_tick = functools.partial(tick, lo + 1, i, *ks[1])
                return next_tick() if body is None else body(i, c, next_tick)

            carry = step(a, carry) if b - a == 1 else lax.fori_loop(a, b, step, carry)
            a = b
        return carry

    def idle(n):
        if n > 0:
            pairs(n // 2)
            if n % 2:
                tick(now[0], 0, kind(now[0]), kind(now[0] + _DEPTH))
                now[0] += 1

    def stream(n, body, carry, ready):
        idle(max(ready(i) - 2 * i for i in range(n)) - now[0])
        return pairs(n, body, carry)

    def aligned(start, size):
        return pl.ds(start if isinstance(start, int) else pl.multiple_of(start, size), size)

    x_copy = pltpu.make_async_copy(x_hbm, x_v, small_sems.at[0])
    wr_copy = pltpu.make_async_copy(wr_hbm, wr_v, small_sems.at[1])
    x_copy.start()
    for g in range(_DEPTH):
        start_step(g, 0, *kind(g))
    wr_copy.start()

    x_copy.wait()
    x = x_v[0].astype(_F32)
    xn = _layernorm(x).astype(_BF16).astype(_F32)
    for j in range(M // _LANES):
        blk = jnp.broadcast_to(xn[:, j * _LANES:(j + 1) * _LANES], (_LANES, _LANES))
        tbl_ref[j * _LANES:(j + 1) * _LANES, :] = blk.T

    for j in range(G):
        idle(1)
        source = lax.broadcasted_iota(jnp.int32, (T, Dc), 0) * G + j
        hit = source == lax.broadcasted_iota(jnp.int32, (T, Dc), 1)
        perm_ref[j * T:(j + 1) * T, :] = jnp.where(hit, 1.0, 0.0).astype(_BF16)

    def q_body(i, acc, next_tick):
        for b in range(tiles // 2):
            if b == tiles // 4:
                next_tick()
            base = pl.multiple_of(i * tiles * G + b * 8, 8)
            xb = tbl_ref[pl.ds(base, 8), :]
            for k in range(8):
                acc = acc + wq_v[base + k].astype(_F32) * xb[k:k + 1, :]
        return acc

    q = stream(M // (tiles * G), q_body, jnp.zeros((H, D), _F32),
               lambda i: wq_ready((i + 1) * tiles * G)).astype(_BF16)

    own_head = (lax.broadcasted_iota(jnp.int32, (H, G * H), 1) % H
                == lax.broadcasted_iota(jnp.int32, (H, G * H), 0))

    def uk_body(i, carry, next_tick):
        full = []
        for k in range(8):
            if k == 4:
                next_tick()
            w = wuk_v[pl.ds((8 * i + k) * G, G)].reshape(G * H, D)
            full.append(lax.dot_general(q, w, _NT, preferred_element_type=_F32))
        z_ref[aligned(i * 8, 8), :] = jnp.concatenate(
            [jnp.sum(jnp.where(own_head, f, 0.0), axis=0, keepdims=True) for f in full], axis=0)
        return carry

    stream(T // 8, uk_body, 0, lambda i: wuk_ready((i + 1) * 8 * G))
    idle(1)
    zt = z_ref[...].T * (D ** -0.5)
    qa = jnp.concatenate([zt[j * H:(j + 1) * H, :] for j in range(G)], axis=1).astype(_BF16)
    idle(1)
    qa = jnp.dot(qa, perm_ref[...], preferred_element_type=_F32).astype(_BF16)

    def score_body(i, peak, next_tick):
        for k in range(2):
            if k == 1:
                next_tick()
            s = lax.dot_general(qa, ckv_v[aligned((2 * i + k) * rows, rows), :], _NT,
                                preferred_element_type=_F32)
            s_ref[2 * i + k] = s
            peak = jnp.maximum(peak, s)
        return peak

    peak = stream(Sk // (2 * rows), score_body, jnp.full((H, rows), -jnp.inf, _F32),
                  lambda i: ckv_ready((i + 1) * 2 * rows))
    peak = jnp.broadcast_to(jnp.max(peak, axis=-1, keepdims=True), (H, rows))

    def value_body(i, total, next_tick):
        acc = acc_ref[...]
        for k in range(4):
            if k == 3:
                next_tick()
            p = jnp.exp(s_ref[4 * i + k] - peak)
            total = total + p
            acc = acc + jnp.dot(p.astype(_BF16), ckv_v[aligned((4 * i + k) * rows, rows), :],
                                preferred_element_type=_F32)
        acc_ref[...] = acc
        return total

    acc_ref[...] = jnp.zeros_like(acc_ref)
    total = pairs(Sk // (4 * rows), value_body, jnp.zeros((H, rows), _F32))
    idle(1)
    lat = acc_ref[...] / jnp.sum(total, axis=-1, keepdims=True)
    z_ref[...] = jnp.concatenate([lat[:, j * T:(j + 1) * T] for j in range(G)], axis=0).T

    def uv_body(i, ctx, next_tick):
        zb = z_ref[aligned(i * tiles, tiles), :]
        for k in range(tiles):
            if k == tiles - 4:
                next_tick()
            lhs = jnp.where(own_head, zb[k:k + 1, :], 0.0).astype(_BF16)
            t = i * tiles + k
            w = jnp.concatenate([wuv_v[j * T + t] for j in range(G)], axis=0)
            ctx = ctx + jnp.dot(lhs, w, preferred_element_type=_F32)
        return ctx

    ctx_ref[...] = stream(T // tiles, uv_body, jnp.zeros((H, D), _F32), lambda i: wuv_ready(Dc))

    heads = tiles * _LANES // M

    def o_body(i, carry, next_tick):
        for k in range(heads):
            if k == heads - 1:
                next_tick()
            lhs = jnp.broadcast_to(ctx_ref[pl.ds(heads * i + k, 1), :], (8, D)).astype(_BF16)
            w = wo_v[aligned((heads * i + k) * D, D), :]
            carry = carry + jnp.dot(lhs, w, preferred_element_type=_F32)
        return carry

    attn = stream(H // heads, o_body, jnp.zeros((8, M), _F32),
                  lambda i: wo_ready((i + 1) * heads * D))

    idle(1)
    h = x + attn[0:1, :]
    hn = _layernorm(h)
    hb = jnp.broadcast_to(hn, (8, M)).astype(_BF16)
    idle(1)
    wr_copy.wait()
    wr = wr_v[...].astype(_F32)
    r = sum(jnp.sum(hn[:, j * _LANES:(j + 1) * _LANES] * wr[j:j + 1, :], axis=-1, keepdims=True)
            for j in range(M // _LANES))
    gate = jax.nn.sigmoid(r)
    resid = h + (hn + hn * 0.0)

    def project(w_v, window):
        return lax.dot_general(hb, w_v[window, :], _NT, preferred_element_type=_F32)

    def silu(v):
        return v * jax.nn.sigmoid(v)

    def up_body(i, carry, next_tick):
        g = silu(project(wg_v, aligned(2 * i * rows, 2 * rows)))
        u0 = project(wu_v, aligned(2 * i * rows, rows))
        next_tick()
        u1 = project(wu_v, aligned((2 * i + 1) * rows, rows))
        act_ref[2 * i] = g[:, :rows] * u0
        act_ref[2 * i + 1] = g[:, rows:] * u1
        return carry

    stream(f_full // 2, up_body, 0, lambda i: wu_ready((i + 1) * 2 * rows))
    idle(wu_ready(F) + 1 - now[0])
    rest = pl.ds(f_full * rows, f_rest)
    act_rest = (silu(project(wg_v, rest)) * project(wu_v, rest)).astype(_BF16)
    y = jnp.zeros((8, M), _F32)
    done = 0
    for edge in (*range(4, f_full, 4), f_full + 1):
        idle(wd_ready(min(edge * rows, F)) + 1 - now[0])
        for i in range(done, edge):
            act, window = ((act_ref[i].astype(_BF16), pl.ds(i * rows, rows)) if i < f_full
                           else (act_rest, rest))
            y = y + jnp.dot(act, wd_v[window, :], preferred_element_type=_F32)
        done = edge
    assert now[0] >= n_steps and f_full % 2 == 0
    o_ref[0] = (resid + y[0:1, :] * gate).astype(o_ref.dtype)


@jax.jit
def pallas_sequential_preLN__compressed_kv_cla__moe_arch_mod__decode_kernel(
    A_x: jax.Array,
    A_c_kv: jax.Array,
    A_w_q: jax.Array,
    A_w_uk: jax.Array,
    A_w_uv: jax.Array,
    A_w_o: jax.Array,
    B_x: jax.Array,
    B_w_r: jax.Array,
    B_w_gate: jax.Array,
    B_w_up: jax.Array,
    B_w_down: jax.Array,
):
    del B_x
    B, Sq, M = A_x.shape
    _, Sk, Dc = A_c_kv.shape
    _, H, D = A_w_q.shape
    F = B_w_gate.shape[1]
    assert B == 1 and Sq == 1 and D == _LANES and Dc == M and Dc * H == _LANES * _LANES

    hbm = pl.BlockSpec(memory_space=pltpu.HBM)
    return pl.pallas_call(
        _kernel,
        out_shape=jax.ShapeDtypeStruct((B, Sq, M), A_x.dtype),
        in_specs=[hbm] * 10,
        out_specs=pl.BlockSpec(memory_space=pltpu.VMEM),
        scratch_shapes=[
            pltpu.VMEM((B, Sq, M), _BF16),
            pltpu.VMEM((M // _LANES, _LANES), _BF16),
            pltpu.VMEM((Sk, Dc), _BF16),
            pltpu.VMEM((M, H, D), _BF16),
            pltpu.VMEM((Dc, H, D), _BF16),
            pltpu.VMEM((Dc, H, D), _BF16),
            pltpu.VMEM((H * D, M), _BF16),
            pltpu.VMEM((F, M), _BF16),
            pltpu.VMEM((F, M), _BF16),
            pltpu.VMEM((F, M), _BF16),
            pltpu.VMEM((M, _LANES), _F32),
            pltpu.VMEM((Dc, Dc), _BF16),
            pltpu.VMEM((_LANES, _LANES), _F32),
            pltpu.VMEM((Sk // _LANES, H, _LANES), _F32),
            pltpu.VMEM((H, Dc), _F32),
            pltpu.VMEM((H, D), _F32),
            pltpu.VMEM((F // _LANES, 8, _LANES), _F32),
            pltpu.SemaphoreType.DMA((2 * pl.next_power_of_2(_DEPTH + 1),)),
            pltpu.SemaphoreType.DMA((2,)),
        ],
        compiler_params=pltpu.CompilerParams(
            vmem_limit_bytes=64 * 2**20,
            disable_bounds_checks=True,
            disable_semaphore_checks=True,
        ),
    )(
        A_x,
        A_c_kv.reshape(Sk, Dc),
        A_w_q,
        A_w_uk,
        A_w_uv,
        A_w_o.reshape(H * D, M),
        B_w_r.reshape(M // _LANES, _LANES),
        B_w_gate.T,
        B_w_up.T,
        B_w_down,
    )
```
